```python
import os as _os
_os.environ.setdefault("JAX_PLATFORMS", "cpu")
import jax
import jax.numpy as jnp

def _softmax(x, axis=-1):
    return jax.nn.softmax(x, axis=axis)
def _gelu(x):
    return jax.nn.gelu(x, approximate=True)
def _silu(x):
    return jax.nn.silu(x)
def _sigmoid(x):
    return jax.nn.sigmoid(x)
def _layernorm(x, axis=-1, eps=1e-5):
    m = jnp.mean(x, axis=axis, keepdims=True)
    v = jnp.var(x, axis=axis, keepdims=True)
    return (x - m) / jnp.sqrt(v + eps)
def _scatter_add(tgt, idx, src, axis=0):
    return tgt.at[idx].add(src)
def _segment_sum(src, seg, n):
    return jax.ops.segment_sum(src, seg, n)
class _Rng:
    def __init__(self, key):
        self._k = key
    def _next(self):
        self._k, sub = jax.random.split(self._k)
        return sub
    def normal(self, shape):
        return jax.random.normal(self._next(), shape, dtype=jnp.bfloat16)
    def randint(self, lo, hi, shape):
        return jax.random.randint(self._next(), shape, lo, hi, dtype=jnp.int32)
    def uniform(self, shape, lo=0.0, hi=1.0):
        return jax.random.uniform(self._next(), shape, jnp.bfloat16, lo, hi)
    def permutation(self, n):
        return jax.random.permutation(self._next(), n)


kernel_name = 'interleave_layers__sliding_local_dilated__glu_gated_reglu__prompt'

def setup_inputs():
    _rng = _Rng(jax.random.key(int.from_bytes(__import__("os").urandom(4), "little")))
    _w = (lambda a: (lambda t: t.astype(jnp.bfloat16) if jnp.issubdtype(t.dtype, jnp.floating) else t)(jnp.asarray(a)))
    def _A_setup():
        B, S, D = 1, 2048, 512
        return {
            "x": _w((lambda *s: _rng.normal(s) * 0.05)(B, S, D)),
            "wqkv": _w((lambda *s: _rng.normal(s) * 0.05)(D, 3 * D)),
            "wo": _w((lambda *s: _rng.normal(s) * 0.05)(D, D)),
        }
    _A_in = _A_setup()

    def _B_setup():
        B, S, D, F = 1, 2048, 512, 1792
        return {
            "x": _w((lambda *s: _rng.normal(s) * 0.05)(B, S, D)),
            "W_gate": _w((lambda *s: _rng.normal(s) * 0.8)(D, F) * (2.0 / D) ** 0.5),
            "W_up": _w((lambda *s: _rng.normal(s) * 0.8)(D, F) * (2.0 / D) ** 0.5),
            "W_down": _w((lambda *s: _rng.normal(s) * 0.8)(F, D) * (1.0 / F) ** 0.5),
        }
    _B_in = _B_setup()

    return {
        "A_x": _A_in["x"],
        "A_wqkv": _A_in["wqkv"],
        "A_wo": _A_in["wo"],
        "B_x": _B_in["x"],
        "B_W_gate": _B_in["W_gate"],
        "B_W_up": _B_in["W_up"],
        "B_W_down": _B_in["W_down"],
    }

def reference(A_x, A_wqkv, A_wo, B_x, B_W_gate, B_W_up, B_W_down):
    def _A_ref(x, wqkv, wo):
        B, S, D = x.shape
        H = 32; Dh = D // H
        W, dil = 8, 2
        qkv = (lambda x, *d: x.transpose(*d))((x @ wqkv).reshape(B, S, 3, H, Dh), 2, 0, 3, 1, 4)
        q, k, v = qkv[0], qkv[1], qkv[2]
        scale = Dh ** -0.5
        pos = jnp.arange(S)
        off = jnp.arange(W) * dil
        idx = pos[:, None] - off[None, :]
        mask = idx >= 0
        idx_c = jnp.where(mask, idx, 0).reshape(-1)
        kg = k[:, :, idx_c, :].reshape(B, H, S, W, Dh)
        vg = v[:, :, idx_c, :].reshape(B, H, S, W, Dh)
        logits = jnp.einsum("bhsd,bhswd->bhsw", q, kg) * scale
        logits = jnp.where(mask[None, None, :, :], logits, -1e9)
        attn = _softmax(logits, axis=-1)
        o = jnp.einsum("bhsw,bhswd->bhsd", attn, vg)
        return (lambda x, *d: x.transpose(*d))(o, 0, 2, 1, 3).reshape(B, S, D) @ wo

    def _B_ref(x, W_gate, W_up, W_down):
        gate = jnp.einsum("bsd,df->bsf", x, W_gate)
        up = jnp.einsum("bsd,df->bsf", x, W_up)
        gate = gate * (lambda x, dt: x.astype(dt))(gate > 0, gate.dtype)
        h = gate * up
        return jnp.einsum("bsf,fd->bsd", h, W_down)

    x = A_x
    x = x + _A_ref(_layernorm(x, axis=-1), A_wqkv, A_wo)
    x = x + _B_ref(_layernorm(x, axis=-1), B_W_gate, B_W_up, B_W_down)
    x = x + _A_ref(_layernorm(x, axis=-1), A_wqkv, A_wo)
    x = x + _B_ref(_layernorm(x, axis=-1), B_W_gate, B_W_up, B_W_down)
    return x
```

```python
import contextlib
import functools
import jax, jax.numpy as jnp, numpy as np
from jax import lax
import jax.experimental.pallas as pl
import jax.experimental.pallas.tpu as pltpu

S, D, F, H, DH, W, DIL = 2048, 512, 1792, 32, 16, 8, 2
HALO = 16
LOG2E = 1.4426950408889634
f32, bf16, i32 = jnp.float32, jnp.bfloat16, jnp.int32
P = functools.partial

def _pk(vals):
    return [pltpu.bitcast(v.astype(bf16), i32) for v in vals]
def _a_ops(a11, a12, a21, a22):
    return [a11 + a22, a21 + a22, a11, a22, a11 + a12, a21 - a11, a12 - a22]
def _b_ops(b11, b12, b21, b22):
    return [b11 + b22, b11, b12 - b22, b21 - b11, b22, b11 + b12, b21 + b22]
def _comb(m):
    m1, m2, m3, m4, m5, m6, m7 = m
    return (m4 - m5) + m1 + m7, m3 + m5, m2 + m4, (m3 - m2) + m1 + m6
ORDER = (1, 3, 2, 4, 0, 5, 6)
def _products(f):
    m = {i: f(i) for i in ORDER}
    return [m[i] for i in range(7)]
def _quad(a):
    m, k = a.shape
    return a[:m//2, :k//2], a[:m//2, k//2:], a[m//2:, :k//2], a[m//2:, k//2:]
def _ops2(X, ops):
    outer = [ops(X[r][c], X[r][2 + c], X[2 + r][c], X[2 + r][2 + c]) for r in range(2) for c in range(2)]
    return [_pk(ops(*[outer[q][i] for q in range(4)])) for i in range(7)]
def _comb2(Pr):
    C = [[None] * 4 for _ in range(4)]
    for q in range(4):
        cc = _comb([Pr[i][q] for i in range(7)])
        for o in range(4):
            C[(o // 2) * 2 + q // 2][(o % 2) * 2 + q % 2] = cc[o]
    return C
def _tiles(a): return [a[:, c:c + 128] for c in range(0, a.shape[1], 128)]
def _sum(xs): return functools.reduce(lambda a, b: a + b, xs)

class _Blk:
    def __init__(self, ref, rows, base=0): self.ref, self.rows, self.base = ref, rows, base
    def _ix(self, idx):
        i, r, c = (idx + (slice(None),) * 2)[:3] if isinstance(idx, tuple) else (idx, slice(None), slice(None))
        a, b, _ = r.indices(self.rows)
        if isinstance(self.base, int): return pl.ds(self.base + i * self.rows + a, b - a), c
        return pl.ds(pl.multiple_of(self.base + (i * self.rows + a), 8), b - a), c
    def __getitem__(self, idx): return self.ref[self._ix(idx)]
    def __setitem__(self, idx, v): self.ref[self._ix(idx)] = v

class _Mxu:
    def __init__(self, never=None): self.t, self.steps, self.never, self.done, self.now = 0.0, [], never, [], 0.0
    def spread(self, tasks, t0, t1):
        tot = sum(w for w, _, _ in tasks); acc = 0
        for w, leads, f in tasks:
            acc += w
            t = self.t + t0 + (t1 - t0) * acc / tot
            g = f()
            self.steps += [(t - lead, g) for lead in leads + (0,)]
        self.steps.sort(key=lambda p: p[0])
    def flush(self):
        for _, g in self.steps: next(g)
        self.steps = []
    def dot(self, a, b):
        n = a.shape[0] // 8
        dur = a.shape[0] * 2 * (a.shape[1] // 128) * (b.shape[1] // 128) / 4
        pins = {}
        while self.steps and self.steps[0][0] < self.t + dur:
            self.now, g = self.steps.pop(0)
            pins.setdefault(max(0, int((self.now - self.t) / dur * n)), []).extend(next(g) or [])
        if any(pins.values()):
            rows = []
            for g in range(n):
                blk = a[g * 8:(g + 1) * 8]
                if pins.get(g):
                    p = functools.reduce(jnp.bitwise_or, [p if p.dtype == i32 else pltpu.bitcast(p, i32) for p in pins[g]])
                    v = jnp.where(self.never, p, blk[:, :128])
                    blk = v if blk.shape[1] == 128 else jnp.concatenate([v, blk[:, 128:]], 1)
                rows.append(blk)
            a = jnp.concatenate(rows, 0)
        out = jnp.dot(pltpu.bitcast(a, bf16), pltpu.bitcast(b, bf16), preferred_element_type=f32)
        self.done += [(self.t + 110 + 8 * r, out, r) for r in range(0, 2 * n, 4)]
        self.t += dur
        return out
    def after(self, v):
        ready = [d for d in self.done if d[0] <= self.now]
        if not ready: return v
        _, out, r = max(ready, key=lambda d: d[0])
        return jnp.where(self.never, out[r * 8:(r + 1) * 8, :128], v)

def _once(f, *args):
    def g(): yield f(*args)
    return g

def make(T=512, flag=None, a0=400, a1=16400, l0=700, l1=5200, m0=800, m1=5200, prof=False, lead0=400, lead1=150,
         ll0=700, ll1=350, only=None, tl=6000, tlead=250, pf=0.4):
    sc_ = jax.named_scope if prof else (lambda n: contextlib.nullcontext())
    flags = {flag: True} if flag else None
    nT = S // T; M = T // 2; Q = T // 4; nV = 2 * nT; sc = T / 512; NB = 4

    def kern(x_hbm, wqkv_hbm, wo_hbm, wg_hbm, wu_hbm, wd_hbm, o_hbm,
             xs, rqkv, ro, rg, ru, rd, wtmp, tqkv, to, tgu, td2, td1,
             qb, kb, vb, hq_ref, ho, hf, hd, hd1, x1, zero, sem, osem):
        tqkv, to, tgu, td2, td1 = _Blk(tqkv, 128), _Blk(to, 128), _Blk(tgu, 64), _Blk(td2, 192), _Blk(td1, 64)
        hq = lambda v: _Blk(hq_ref, M // 2, (v % NB) * (7 * M // 2))
        ho, hf, hd = _Blk(ho, M // 2), _Blk(hf, Q // 2), _Blk(hd, Q // 2)
        def mxu(): return _Mxu(zero[...] != 0)
        def cp_x(t): return pltpu.make_async_copy(x_hbm.at[pl.ds(t * T, T)], xs.at[pl.ds(t * T, T)], sem.at[t])
        def cp_qkv(j): return pltpu.make_async_copy(wqkv_hbm.at[:, pl.ds(j * D, D)], rqkv.at[j], sem.at[nT + j])
        def cp_o(): return pltpu.make_async_copy(wo_hbm, ro, sem.at[nT + 3])
        def cp_g(): return pltpu.make_async_copy(wg_hbm, rg, sem.at[nT + 4])
        def cp_u(): return pltpu.make_async_copy(wu_hbm, ru, sem.at[nT + 5])
        def cp_d(): return pltpu.make_async_copy(wd_hbm, rd, sem.at[nT + 6])
        def cp_out(t):
            r = pl.ds(pl.multiple_of(t * T, T), T)
            return pltpu.make_async_copy(xs.at[r], o_hbm.at[r], osem.at[t])
        order = [cp_x(0), cp_qkv(0), cp_qkv(1), cp_qkv(2), cp_x(1), cp_o(), cp_x(2), cp_g(), cp_u(), cp_d()] + [cp_x(t) for t in range(3, nT)]
        for c in order: c.start()
        zero[...] = jnp.zeros(zero.shape, i32)

        def prep_qkv(j, g):
            lane = lax.broadcasted_iota(i32, (8, 128), 1)
            dd, sub, hh = lane // 32, (lane // 8) % 4, lane % 8
            src = []
            for r0 in (g * 16, 256 + g * 16):
                w = pltpu.bitcast(rqkv[j, r0:r0 + 16, :], i32)
                src.append([jnp.take_along_axis(w[:, t * 128:(t + 1) * 128], hh * 16 + ((sub - t) % 4) * 4 + dd, axis=1) for t in range(4)])
            yield
            cols = []
            for half in src:
                for i in range(4):
                    o = half[3]
                    for t in range(3):
                        o = jnp.where(sub == (t + i) % 4, half[t], o)
                    cols.append(pltpu.roll(o, 128 - 8 * i, 1) if i else o)
            yield
            top, bot = [pltpu.bitcast(jnp.concatenate(c, axis=1), bf16).astype(f32) for c in (cols[:4], cols[4:])]
            for i, b in enumerate(_pk(_b_ops(top[:, :256], top[:, 256:], bot[:, :256], bot[:, 256:]))):
                tqkv[j * 7 + i, g * 8:(g + 1) * 8] = b
            yield [c for i in range(7) for c in _tiles(tqkv[j * 7 + i, g * 8:(g + 1) * 8])]
        def qkv_tasks(j): return [(1, (300, 150), P(prep_qkv, j, g)) for g in range(16)]
        def stage_o(g):
            w = ro[g * 64:(g + 1) * 64, :].astype(f32)
            for t in range(4):
                wtmp[t, g * 64:(g + 1) * 64, :] = w[:, t * 128:(t + 1) * 128]
            return [wtmp[t, g * 64:g * 64 + 8, :] for t in range(4)]
        def prep_o(i, g, e):
            def rows(i, t):
                return jnp.concatenate([wtmp[t, pl.ds(a * 128 + 4 * i + (g if a + i < 4 else (g + 1) % 4), 8, stride=16), :] for a in (2 * e, 2 * e + 1)], axis=0)
            r = slice(i * 64 + g * 16 + e * 8, i * 64 + g * 16 + e * 8 + 8)
            for t in range(2):
                for n, b in enumerate(_pk(_b_ops(rows(i, t), rows(i, 2 + t), rows(2 + i, t), rows(2 + i, 2 + t)))):
                    to[n, r, t * 128:(t + 1) * 128] = b
            return [c for n in (0, 5, 6) for c in _tiles(to[n, r])]
        def prep2(get, dst, ix):
            ops = _ops2([[get(r, n) for n in range(4)] for r in range(4)], _b_ops)
            for i in range(7):
                for j in range(7): dst[ix(i, j)] = ops[i][j]
            return [dst[ix(i, j)] for i in (0, 2, 3, 5, 6) for j in (5, 6)]
        def prep_gu(ref, s, c, g):
            ix = lambda i, j: (i * 7 + j, slice(g * 8, (g + 1) * 8), slice(c * 256 + s * 128, c * 256 + (s + 1) * 128))
            return prep2(lambda r, n: ref[r * 128 + g * 16:r * 128 + (g + 1) * 16, c * 512 + n * 128:c * 512 + (n + 1) * 128].astype(f32), tgu, ix)
        def prep_gu_tail(g):
            lo = lax.broadcasted_iota(i32, (8, 128), 1) < 64
            X = []
            for r in range(4):
                a, b = [pltpu.bitcast(ref[r * 128 + g * 16:r * 128 + (g + 1) * 16, 1536:1792], i32) for ref in (rg, ru)]
                X.append([(a, b, pltpu.roll(a, 64, 1), pltpu.roll(b, 64, 1)) for a, b in zip(_tiles(a), _tiles(b))])
            yield
            X = [_tiles(pltpu.bitcast(jnp.concatenate([z for a, b, ra, rb in row for z in (jnp.where(lo, a, rb), jnp.where(lo, ra, b))], 1), bf16).astype(f32)) for row in X]
            yield prep2(lambda r, n: X[r][n], tgu, lambda i, j: (i * 7 + j, slice(g * 8, (g + 1) * 8), slice(768, 896)))
        def prep_d(c, g):
            ix = lambda i, j: (i, slice(c * 64 + g * 8, c * 64 + (g + 1) * 8), slice(j * 128, (j + 1) * 128))
            return prep2(lambda r, n: rd[c * 512 + r * 128 + g * 16:c * 512 + r * 128 + (g + 1) * 16, n * 128:(n + 1) * 128].astype(f32), td2, ix)
        def prep_d_tail(g):
            top = rd[1536 + g * 16:1536 + (g + 1) * 16, :].astype(f32); bot = rd[1664 + g * 16:1664 + (g + 1) * 16, :].astype(f32)
            ops = _pk(_b_ops(top[:, :256], top[:, 256:], bot[:, :256], bot[:, 256:]))
            for i, b in enumerate(ops): td1[i, g * 8:(g + 1) * 8] = b
            return [td1[i, g * 8:(g + 1) * 8, :128] for i in range(7)]

        def xrows(t, r0, n):
            return pl.ds(t * T + r0, n) if isinstance(t, int) else pl.ds(pl.multiple_of(t * T + r0, n), n)
        def norm_tasks(mx, get, parts, finish):
            tasks = []
            def rows(hs, p, e, r0):
                x = get(r0)
                xt = _tiles(x)
                mean = jnp.sum(mx.after(xt[0]) + xt[1] + xt[2] + xt[3], axis=-1, keepdims=True) * (1.0 / D)
                yield
                xc = x - mean
                var = jnp.mean(xc * xc, axis=-1, keepdims=True)
                yield
                hs[p, e] = xc * lax.rsqrt(var + 1e-5)
                yield _tiles(hs[p, e])[:1]
            for u in range(T // parts // 16):
                hs = {}
                for p in range(parts):
                    for e in range(2):
                        tasks.append((30, (ll0, ll1), P(rows, hs, p, e, p * (T // parts) + u * 16 + e * 8)))
                tasks.append((10 * parts, (), _once(lambda hs, u: finish(u, [jnp.concatenate([hs[p, 0], hs[p, 1]], 0) for p in range(parts)]), hs, u)))
            return tasks
        def put1(dst, u, bands):
            top, bot = bands
            ops = _pk(_a_ops(top[:, :256], top[:, 256:], bot[:, :256], bot[:, 256:]))
            for i, a in enumerate(ops): dst[i, u * 8:(u + 1) * 8] = a
            return [c for i in range(7) for c in _tiles(dst[i, u * 8:(u + 1) * 8])]
        def ln1_tasks(mx, v):
            return norm_tasks(mx, lambda r0: xs[xrows(v % nT, r0, 8), :].astype(f32), 2, P(put1, hq(v)))
        def qkv(mx, j, v):
            src = hq(v); s0 = (v % NB) * 4
            C = _comb(_products(lambda i: mx.dot(src[i], tqkv[j * 7 + i])))
            for o in range(4):
                r0 = (o // 2) * M
                for t in range(2):
                    val = C[o][:, t * 128:(t + 1) * 128]
                    lt = s0 + (o % 2) * 2 + t
                    if j == 0: qb[lt, r0:r0 + M, :] = val * (DH ** -0.5 * LOG2E)
                    elif j == 1: kb[lt, HALO + r0:HALO + r0 + M, :] = val
                    else: vb[lt, HALO + r0:HALO + r0 + M, :] = val
        def attn_tasks(mx, v):
            s0, s1 = (v % NB) * 4, ((v + 1) % NB) * 4
            def rows(dst, key, r0):
                q = [qb[s0 + t, r0:r0 + 8, :] for t in range(4)]
                q[0] = mx.after(q[0])
                lg = [_sum([q[t] * kb[s0 + t, pl.ds(HALO + r0 - DIL * w, 8), :] for t in range(4)]) for w in range(W)]
                rot = [[pltpu.roll(s, a, 1) for a in (32, 64, 96)] for s in lg]
                yield
                lg = [(s + r[0]) + (r[1] + r[2]) for s, r in zip(lg, rot)]
                yield
                edge = r0 < HALO
                if edge:
                    pos = lax.broadcasted_iota(i32, (8, 128), 0) + ((v % nT) * T + r0)
                    lg = [jnp.where(pos >= DIL * w, s, -1e9 * LOG2E) if w else s for w, s in enumerate(lg)]
                m = functools.reduce(jnp.maximum, lg)
                p = [jnp.exp2(s - m) for s in lg]
                inv = 1.0 / _sum(p)
                out = []
                for t in range(4):
                    val = [vb[s0 + t, pl.ds(HALO + r0 - DIL * w, 8), :] for w in range(W)]
                    if edge:
                        val = [jnp.where(pos >= DIL * w, z, vb[s0 + t, HALO:HALO + 1, :]) if w else z for w, z in enumerate(val)]
                    out.append(_sum([a * z for a, z in zip(p, val)]) * inv)
                dst[key] = jnp.concatenate(out, 1)
                yield out
            def halo():
                for t in range(4):
                    kb[s1 + t, 0:HALO, :] = kb[s0 + t, T:T + HALO, :]
                    vb[s1 + t, 0:HALO, :] = vb[s0 + t, T:T + HALO, :]
            tasks = []
            for u in range(M // 16):
                os_ = {}
                for p in range(2):
                    for e in range(2):
                        tasks.append((162, (lead0, lead1), P(rows, os_, (p, e), p * M + u * 16 + e * 8)))
                tasks.append((34, (), _once(lambda os_, u: put1(ho, u, [jnp.concatenate([os_[p, 0], os_[p, 1]], 0) for p in range(2)]), os_, u)))
            return tasks + [(1, (), _once(halo))]
        def proj(mx, t):
            C = _comb(_products(lambda i: mx.dot(ho[i], to[i])))
            c = jnp.concatenate([jnp.concatenate(C[:2], 1), jnp.concatenate(C[2:], 1)], 0)
            x = xs[xrows(t, 0, T), :].astype(f32)
            def get(r0):
                y = x[r0:r0 + 8] + c[r0:r0 + 8]
                x1[r0:r0 + 8, :] = y
                return y
            def finish(u, bands):
                ops = _ops2([_tiles(b) for b in bands], _a_ops)
                for i in range(7):
                    for j in range(7):
                        hf[i, u * 8:(u + 1) * 8, j * 128:(j + 1) * 128] = ops[i][j]
                return [hf[i, u * 8:(u + 1) * 8, j * 128:(j + 1) * 128] for i in range(7) for j in (0, 5, 6)]
            return norm_tasks(mx, get, 4, finish)
        def ffn(mx, t):
            def chunk(c0):
                return _comb2(_products(lambda i: _comb(_products(
                    lambda j: mx.dot(hf[i, :, j * 128:(j + 1) * 128], tgu[i * 7 + j, :, c0:c0 + 128])))))
            lo = lax.broadcasted_iota(i32, (16, 128), 1) < 64
            def tail_rows(C, u):
                act = []
                for r in range(4):
                    row = []
                    for p in range(2):
                        a, b = C[r][2 * p][u * 16:(u + 1) * 16], C[r][2 * p + 1][u * 16:(u + 1) * 16]
                        row.append((a, b, pltpu.roll(a, 64, 1), pltpu.roll(b, 64, 1)))
                    act.append(row)
                yield
                act = [[jnp.maximum(jnp.where(lo, a, rb), 0.0) * jnp.where(lo, ra, b) for a, b, ra, rb in row] for row in act]
                pins = []
                for r in range(2):
                    for i, a in enumerate(_pk(_a_ops(act[r][0], act[r][1], act[2 + r][0], act[2 + r][1]))):
                        ix = (slice(r * Q // 2 + u * 8, r * Q // 2 + (u + 1) * 8), slice(i * 128, (i + 1) * 128))
                        hd1[ix] = a
                        pins.append(hd1[ix])
                yield pins
            C = chunk(768)
            mx.spread([(1, (tlead,), P(tail_rows, C, u)) for u in range(Q // 16)], 300 * sc, tl * sc)
            for c in range(3):
                G = chunk(c * 256); U = chunk(c * 256 + 128)
                act = [[jnp.maximum(g, 0.0) * u for g, u in zip(gr, ur)] for gr, ur in zip(G, U)]
                for i, row in enumerate(_ops2(act, _a_ops)):
                    for j, a in enumerate(row):
                        hd[i * 7 + j, :, c * 128:(c + 1) * 128] = a
            def outer(i):
                cc = _comb(_products(lambda j: mx.dot(hd[i * 7 + j], td2[i, :, j * 128:(j + 1) * 128])))
                r = _quad(mx.dot(hd1[:, i * 128:(i + 1) * 128], td1[i]))
                return [cc[q] + r[q] for q in range(4)]
            C = _comb2(_products(outer))
            mx.flush()
            for r in range(4):
                y = x1[r * Q:(r + 1) * Q, :] + jnp.concatenate(C[r], 1)
                xs[xrows(t, r * Q, Q), :] = y.astype(bf16)
        def run(tasks, dur):
            mx = _Mxu(); mx.spread(tasks, 0, dur); mx.flush()

        def prologue():
            A = 1792 * sc
            for t in range(4):
                kb[t, 0:HALO, :] = jnp.zeros((HALO, 128), f32)
                vb[t, 0:HALO, :] = jnp.zeros((HALO, 128), f32)
            with sc_("w0"): cp_x(0).wait()
            with sc_("B0"): run(ln1_tasks(_Mxu(), 0), 1500 * sc)
            with sc_("w1"): cp_qkv(0).wait()
            with sc_("B1"):
                run(qkv_tasks(0), 300)
                qkv(mxu(), 0, 0)
            with sc_("w2"): cp_qkv(1).wait(); cp_qkv(2).wait()
            with sc_("B2"):
                run(qkv_tasks(1), 300)
                mx = mxu()
                mx.spread(qkv_tasks(2), 300, A - 100)
                qkv(mx, 1, 0); mx.flush(); qkv(mx, 2, 0)
            with sc_("w3"): cp_x(1).wait(); cp_o().wait(); cp_x(2).wait()
            with sc_("B3"):
                run(ln1_tasks(_Mxu(), 1), 1500 * sc)
                mx = mxu()
                mx.spread(attn_tasks(mx, 0), 300, 3 * A - 50)
                mx.spread([(1, (), _once(stage_o, g)) for g in range(8)] + [(0.5, (), _once(prep_o, i, g, e)) for i in range(2) for g in range(4) for e in range(2)], 0, 3 * A - 100)
                for j in range(3): qkv(mx, j, 1)
                mx.flush()
            prep = [(1, (), _once(prep_gu, ref, s, c, g)) for s, ref in enumerate((rg, ru)) for c in range(3) for g in range(8)]
            prep += [(1, (200,), P(prep_gu_tail, g)) for g in range(8)]
            prep += [(1, (), _once(prep_d, c, g)) for c in range(3) for g in range(8)] + [(0.3, (), _once(prep_d_tail, g)) for g in range(8)]
            n = int(pf * 84)
            with sc_("w4"): cp_g().wait(); cp_u().wait()
            with sc_("B4"):
                mx = mxu()
                mx.spread(ln1_tasks(mx, 2), 300, A - 50)
                mx.spread(prep[:n], 0, 2 * A - 50)
                ln2 = proj(mx, 0)
                mx.spread(ln2, 500, A + 200)
                qkv(mx, 0, 2); mx.flush()
            with sc_("w5"):
                cp_d().wait()
                for t in range(3, nT): cp_x(t).wait()
            with sc_("B5"):
                mx = mxu()
                mx.spread(ln1_tasks(mx, 3), 300, 2 * A - 50)
                mx.spread(prep[n:], 0, 2 * A - 50)
                qkv(mx, 1, 2); qkv(mx, 2, 2); mx.flush()
        if only != 'loop': prologue()
        else:
            for c in order: c.wait()

        def body(v, carry):
            mx = mxu()
            mx.spread(attn_tasks(mx, v), a0 * sc, a1 * sc)
            with sc_('X'): ffn(mx, (v - 1) % nT)
            @pl.when(v > nT)
            def _(): cp_out(v - 1 - nT).start()
            @pl.when(v < nV - 2)
            def _():
                with sc_('Y'):
                    mx = mxu()
                    ln2 = proj(mx, v % nT)
                    mx.spread(ln2, m0 * sc, m1 * sc)
                    mx.spread(ln1_tasks(mx, v + 3), l0 * sc, l1 * sc)
                    for j in range(3): qkv(mx, j, v + 2)
                    mx.flush()
            @pl.when((v >= nV - 2) & (v < nV))
            def _():
                if only != 'loop': run(proj(mxu(), v % nT), 1500 * sc)
            return carry
        if only != 'pro':
            lax.fori_loop(1, nV + 1, body, 0)
        else:
            for t in range(nT): cp_out(t).start()
        for t in range(nT): cp_out(t).wait()

    def fn(A_x, A_wqkv, A_wo, B_x, B_W_gate, B_W_up, B_W_down):
        V = pltpu.VMEM
        out = pl.pallas_call(
            kern,
            in_specs=[pl.BlockSpec(memory_space=pl.ANY)] * 6,
            out_specs=pl.BlockSpec(memory_space=pl.ANY),
            out_shape=jax.ShapeDtypeStruct((S, D), A_x.dtype),
            scratch_shapes=[
                V((S, D), bf16), V((3, D, D), bf16), V((D, D), bf16), V((D, F), bf16), V((D, F), bf16), V((F, D), bf16),
                V((4, D, 128), f32), V((21 * 128, 256), i32), V((7 * 128, 256), i32),
                V((49 * 64, 896), i32), V((7 * 192, 896), i32), V((7 * 64, 256), i32),
                V((NB * 4, T, 128), f32), V((NB * 4, T + HALO, 128), f32), V((NB * 4, T + HALO, 128), f32),
                V((NB * 7 * M // 2, 256), i32), V((7 * M // 2, 256), i32), V((7 * Q // 2, 896), i32), V((49 * Q // 2, 384), i32), V((M // 2, 896), i32), V((T, D), f32),
                V((8, 128), i32),
                pltpu.SemaphoreType.DMA((nT + 7,)), pltpu.SemaphoreType.DMA((nT,))],
            compiler_params=pltpu.CompilerParams(vmem_limit_bytes=110 * 2**20, disable_bounds_checks=True, flags=flags),
        )(A_x.reshape(S, D), A_wqkv, A_wo, B_W_gate, B_W_up, B_W_down)
        return out.reshape(A_x.shape)
    return fn


@jax.jit
def pallas_interleave_layers__sliding_local_dilated__glu_gated_reglu__prompt_kernel(
        A_x, A_wqkv, A_wo, B_x, B_W_gate, B_W_up, B_W_down):
    return make()(A_x, A_wqkv, A_wo, B_x, B_W_gate, B_W_up, B_W_down)
```

```python
import functools

import jax
import jax.numpy as jnp
from jax import lax
import jax.experimental.pallas as pl
import jax.experimental.pallas.tpu as pltpu

S, D, F = 2048, 512, 1792
DH, WIN, DIL = 16, 8, 2
EPS, MASKED = 1e-5, -1e9
LOG2E = 1.4426950408889634
T = 512
M, Q = T // 2, T // 4
NT = S // T
NV = 2 * NT
HALO = 16
f32, bf16, i32 = jnp.float32, jnp.bfloat16, jnp.int32
partial = functools.partial


def _lhs_ops(a11, a12, a21, a22):
    return [a11 + a22, a21 + a22, a11, a22, a11 + a12, a21 - a11, a12 - a22]


def _rhs_ops(b11, b12, b21, b22):
    return [b11 + b22, b11, b12 - b22, b21 - b11, b22, b11 + b12, b21 + b22]


def _strassen(product, order):
    m = {i: product(i) for i in order}
    return jnp.block([[(m[3] - m[4]) + m[0] + m[6], m[2] + m[4]],
                      [m[1] + m[3], (m[2] - m[1]) + m[0] + m[5]]])


def _halves(*rows):
    return [h for r in rows for h in (r[:, :r.shape[1] // 2], r[:, r.shape[1] // 2:])]


def _two_level(ops, rows):
    top, bot = ops(*_halves(rows[0], rows[2])), ops(*_halves(rows[1], rows[3]))
    return [partial(lambda t, b: jnp.concatenate(ops(*_halves(t, b)), axis=1), t, b)
            for t, b in zip(top, bot)]


def _pack(x):
    return pltpu.bitcast(x.astype(bf16), i32)


def _tiles(x):
    return [x[:, c:c + 128] for c in range(0, x.shape[1], 128)]


def _span(i, n, start=0, size=None):
    at = i * n + start
    return pl.ds(at if isinstance(at, int) else pl.multiple_of(at, 8), n if size is None else size)


class _Stream:
    def __init__(self, never=None):
        self.never, self.clock, self.now, self.steps, self.results = never, 0.0, 0.0, [], []

    def spread(self, tasks, start, end):
        total, done = sum(w for w, _, _ in tasks), 0
        for weight, leads, make in tasks:
            done += weight
            due = self.clock + start + (end - start) * done / total
            slot = (end - start) * weight / total
            gen = make()
            self.steps += [(due - (lead * slot if lead < 1 else lead), gen) for lead in leads + (0,)]
        self.steps.sort(key=lambda step: step[0])

    def finish(self):
        for _, gen in self.steps:
            next(gen)
        self.steps = []

    def dot(self, a, b):
        n = a.shape[0] // 8
        cycles = a.shape[0] * (a.shape[1] // 128) * (b.shape[1] // 128) / 2
        ties = {}
        while self.steps and self.steps[0][0] < self.clock + cycles:
            self.now, gen = self.steps.pop(0)
            for v in next(gen) or []:
                ties.setdefault(max(0, int((self.now - self.clock) / cycles * n)), []).append(v)
        if ties:
            rows, at = [], 0
            for g in sorted(ties):
                bits = functools.reduce(
                    jnp.bitwise_or, [v if v.dtype == i32 else pltpu.bitcast(v, i32) for v in ties[g]])
                row = jnp.where(self.never, bits, a[g * 8:g * 8 + 8, :128])
                if a.shape[1] > 128:
                    row = jnp.concatenate([row, a[g * 8:g * 8 + 8, 128:]], axis=1)
                rows += ([a[at:g * 8]] if at < g * 8 else []) + [row]
                at = g * 8 + 8
            a = jnp.concatenate(rows + ([a[at:]] if at < n * 8 else []), axis=0)
        out = jnp.dot(pltpu.bitcast(a, bf16), pltpu.bitcast(b, bf16), preferred_element_type=f32)
        self.results += [(self.clock + 110 + 8 * r, out, r) for r in range(0, 2 * n, 4)]
        self.clock += cycles
        return out

    def not_before(self, x):
        ready = [r for r in self.results if r[0] <= self.now]
        if not ready:
            return x
        _, out, r = max(ready, key=lambda res: res[0])
        return jnp.where(self.never, out[r * 8:r * 8 + 8, :128], x)


def _step(weight, fn, *args):
    def gen():
        yield fn(*args)
    return weight, (), gen


def _merge(a, b):
    def keyed(tasks):
        total, done = sum(w for w, _, _ in tasks), 0
        for task in tasks:
            done += task[0]
            yield (done - task[0] / 2) / total, task
    return [task for _, task in sorted([*keyed(a), *keyed(b)], key=lambda kt: kt[0])]


def _run(tasks, cycles):
    plain = _Stream()
    plain.spread(tasks, 0, cycles)
    plain.finish()


_SEVEN_STEPS = tuple(k / 7 for k in range(6, 0, -1))
_IN_ORDER = (0, 1, 2, 5, 3, 4, 6)
_PAIRS_FIRST = (1, 3, 2, 4, 0, 5, 6)


def _put_one_level(ops, dst, block, n, u, top, bot):
    for i, v in enumerate(ops(*_halves(top, bot))):
        dst[_span(block + i, n, u * 8, 8), :] = _pack(v)
    return [t for i in range(7) for t in _tiles(dst[_span(block + i, n, u * 8, 8), :])]


def _put_two_level(ops, order, dst, block, n, at, rows):
    inner = _two_level(ops, rows)
    for i in order:
        dst[_span(block + i, n, at, 8), :] = _pack(inner[i]())
        yield _tiles(dst[_span(block + i, n, at, 8), 640:])


def _kernel(x_hbm, wqkv_hbm, wo_hbm, wg_hbm, wu_hbm, wd_hbm, out_hbm,
            xs, x_mid, raw_qkv, raw_o, raw_g, raw_u, raw_d, wo_rows,
            w_qkv, w_o, w_gu, w_dn, w_dt, h_qkv, h_o, h_gu, h_dn, h_dt,
            q_buf, k_buf, v_buf, zeros, sem):
    copy = pltpu.make_async_copy
    get_x = lambda t: copy(x_hbm.at[pl.ds(t * T, T)], xs.at[pl.ds(t * T, T)], sem.at[t])
    get_qkv = lambda j: copy(wqkv_hbm.at[:, pl.ds(j * D, D)], raw_qkv.at[j], sem.at[4 + j])
    get_o, get_d = copy(wo_hbm, raw_o, sem.at[2]), copy(wd_hbm, raw_d, sem.at[3])
    get_g, get_u = copy(wg_hbm, raw_g, sem.at[7]), copy(wu_hbm, raw_u, sem.at[7])
    put_x = lambda t: copy(xs.at[_span(t, T)], out_hbm.at[_span(t, T)], sem.at[8])
    for c in (get_qkv(0), get_x(0), get_qkv(1), get_qkv(2), get_x(1), get_x(2),
              get_o, get_g, get_u, get_d, get_x(3)):
        c.start()
    zeros[...] = jnp.zeros(zeros.shape, i32)
    stream = lambda: _Stream(zeros[...] != 0)

    def qkv_weight_tasks(j):
        lane = lax.broadcasted_iota(i32, (D // 2, 128), 1)
        group, eighth, head = lane // 32, (lane // 8) % 4, lane % 8
        src = [jnp.take_along_axis(w, head * DH + ((eighth - a) % 4) * 4 + group, axis=1)
               for a, w in enumerate(_tiles(pltpu.bitcast(raw_qkv[j], i32)))]
        cols = []
        for i in range(4):
            col = src[3]
            for a in range(3):
                col = jnp.where(eighth == (a + i) % 4, src[a], col)
            cols.append(pltpu.roll(col, 128 - 8 * i, 1) if i else col)
        words = jnp.concatenate(cols, axis=1)
        band = lambda r: pltpu.bitcast(words[r:r + 8], bf16).astype(f32)
        vregs = lambda w: [w[r:r + 8] for r in range(0, D // 2, 8)]
        build = lambda u: _put_one_level(_rhs_ops, w_qkv, j * 7, 128, u, band(u * 8), band(128 + u * 8))
        return ([_step(200, vregs, w) for w in src] + [_step(100, vregs, w) for w in cols[1:]]
                + [_step(25, build, u) for u in range(16)])

    def out_weight_tasks():
        def stage(g):
            for h in range(g * 4, g * 4 + 4):
                wo_rows[:, h * 17:h * 17 + DH, :] = jnp.stack(
                    _tiles(raw_o[h * DH:(h + 1) * DH, :].astype(f32)))
            return [wo_rows[t, g * 68:g * 68 + 8, :] for t in range(4)]

        def band(i, group, e):
            dim = lambda a: 4 * i + (group if a + i < 4 else (group + 1) % 4)
            return jnp.block([[wo_rows[t, pl.ds(a * 8 * 17 + dim(a), 8, stride=17), :] for t in range(4)]
                              for a in (2 * e, 2 * e + 1)])

        def build(i, group, e):
            return _put_one_level(_rhs_ops, w_o, 0, 128, i * 8 + group * 2 + e,
                                  band(i, group, e), band(2 + i, group, e))[10:]

        return ([_step(50, stage, g) for g in range(8)]
                + [_step(40, build, i, group, e) for i in range(2) for group in range(4) for e in range(2)])

    def ffn_weight_tasks():
        put = partial(_put_two_level, _rhs_ops, (1, 5, 2, 4, 0, 3, 6))

        def gate_up(ref, block, c, u):
            return put(w_gu, block * 7, 64, u * 8,
                       [ref[_span(r, 128, u * 16, 16), _span(c, 512)].astype(f32) for r in range(4)])

        def gate_up_tail(u):
            low = lax.broadcasted_iota(i32, (8, 128), 1) < 64
            load = lambda ref, r: _tiles(pltpu.bitcast(ref[_span(r, 128, u * 16, 16), 1536:], i32))
            rows = [[(g, up, pltpu.roll(g, 64, 1), pltpu.roll(up, 64, 1))
                     for g, up in zip(load(raw_g, r), load(raw_u, r))] for r in range(4)]
            yield
            rows = [jnp.concatenate([z for g, up, rg, ru in row
                                     for z in (jnp.where(low, g, ru), jnp.where(low, rg, up))], axis=1)
                    for row in rows]
            yield from put(w_gu, 6 * 7, 64, u * 8, [pltpu.bitcast(row, bf16).astype(f32) for row in rows])

        def down(c, u):
            return put(w_dn, 0, 192, c * 64 + u * 8,
                       [raw_d[_span(c * 4 + r, 128, u * 16, 16), :].astype(f32) for r in range(4)])

        def down_tail(u):
            top, bot = [raw_d[_span(r, 128, u * 16, 16), :].astype(f32) for r in (12, 13)]
            return _put_one_level(_rhs_ops, w_dt, 0, 64, u, top, bot)[::2]

        return ([(200, _SEVEN_STEPS, partial(gate_up, ref, 2 * c + s, c, u))
                 for s, ref in enumerate((raw_g, raw_u)) for c in range(3) for u in range(8)]
                + [(200, (300,) + _SEVEN_STEPS, partial(gate_up_tail, u)) for u in range(8)],
                [(200, _SEVEN_STEPS, partial(down, c, u)) for c in range(3) for u in range(8)]
                + [_step(60, down_tail, u) for u in range(8)])

    def norm_tasks(mx, load, parts, last):
        def rows(normed, r):
            x = load(r)
            lanes = _tiles(x)
            mean = jnp.sum(mx.not_before(lanes[0]) + lanes[1] + lanes[2] + lanes[3],
                           axis=-1, keepdims=True) * (1.0 / D)
            yield
            x = x - mean
            var = jnp.sum(x * x, axis=-1, keepdims=True) * (1.0 / D)
            yield
            normed[r] = x * lax.rsqrt(var + EPS)
            yield [normed[r][:, :128]]

        def bands(normed, starts):
            return [jnp.concatenate([normed[s], normed[s + 8]], axis=0) for s in starts]

        tasks = []
        for u in range(T // parts // 16):
            normed = {}
            starts = [p * (T // parts) + u * 16 for p in range(parts)]
            tasks += [(30, (450, 180), partial(rows, normed, r)) for s in starts for r in (s, s + 8)]
            tasks.append(last(u, partial(bands, normed, starts)))
        return tasks

    def norm1_tasks(mx, v):
        t = v % NT
        put = lambda u, bands: _put_one_level(_lhs_ops, h_qkv, t * 7, M // 2, u, *bands())
        return norm_tasks(mx, lambda r: xs[_span(t, T, r, 8), :].astype(f32), 2, partial(_step, 20, put))

    def norm2_tasks(mx, load):
        def put(u, bands):
            yield from _put_two_level(_lhs_ops, (2, 5, 1, 3, 0, 4, 6), h_gu, 0, Q // 2, u * 8, bands())
        return norm_tasks(mx, load, 4, lambda u, bands: (140, _SEVEN_STEPS, partial(put, u, bands)))

    def qkv_product(mx, v, j, i):
        return mx.dot(h_qkv[_span(v % NT * 7 + i, M // 2), :], w_qkv[_span(j * 7 + i, 128), :])

    def qkv(mx, v, j, have=()):
        y = _strassen(lambda i: have[i] if i in have else qkv_product(mx, v, j, i), _IN_ORDER)
        if j == 0:
            q_buf[v % NT] = jnp.stack(_tiles(y * (DH ** -0.5 * LOG2E)))
        else:
            (k_buf, v_buf)[j - 1][v % NT, :, HALO:, :] = jnp.stack(_tiles(y))

    def attention_tasks(mx, v):
        t, t_next = v % NT, (v + 1) % NT

        def rows(result, r):
            tap = lambda ref, w: ref[t, :, pl.ds(HALO + r - DIL * w, 8), :]
            q = q_buf[t, :, r:r + 8, :]
            q = jnp.concatenate([mx.not_before(q[0])[None], q[1:]], axis=0)
            s = [jnp.sum(q * tap(k_buf, w), axis=0) for w in range(WIN)]
            rolled = [[pltpu.roll(z, shift, 1) for shift in (32, 64, 96)] for z in s]
            yield
            s = jnp.stack([(z + zr[0]) + (zr[1] + zr[2]) for z, zr in zip(s, rolled)])
            yield
            values = [tap(v_buf, w) for w in range(WIN)]
            if r < HALO:
                pos = lax.broadcasted_iota(i32, s.shape, 1) + (t * T + r)
                s = jnp.where(pos >= DIL * lax.broadcasted_iota(i32, s.shape, 0), s, MASKED * LOG2E)
                first = v_buf[t, :, HALO:HALO + 1, :]
                values = [jnp.where(pos[:4] >= DIL * w, z, first) if w else z for w, z in enumerate(values)]
            p = jnp.exp2(s - jnp.max(s, axis=0))
            o = functools.reduce(jnp.add, [p[w] * z for w, z in enumerate(values)])
            o = o * pl.reciprocal(jnp.sum(p, axis=0), full_range=False)
            result[r] = [o[i] for i in range(4)]
            yield result[r]

        def operands(result, u):
            top, bot = [jnp.block([result[r], result[r + 8]]) for r in (u * 16, M + u * 16)]
            return _put_one_level(_lhs_ops, h_o, 0, M // 2, u, top, bot)

        def hand_over():
            for ref in (k_buf, v_buf):
                ref[t_next, :, :HALO, :] = ref[t, :, T:, :]

        tasks = []
        for u in range(M // 16):
            result = {}
            tasks += [(162, (480, 60), partial(rows, result, s + u * 16 + e)) for s in (0, M) for e in (0, 8)]
            tasks.append(_step(34, operands, result, u))
        return tasks, [_step(1, hand_over)]

    def project(mx, v):
        y = _strassen(lambda i: mx.dot(h_o[_span(i, M // 2), :], w_o[_span(i, 128), :]), _IN_ORDER)
        y = xs[_span(v % NT, T), :].astype(f32) + y

        def load(r):
            x_mid[r:r + 8, :] = y[r:r + 8]
            return y[r:r + 8]
        return load

    def project_and_norm(mx, v):
        t, n, ys = v % NT, Q // 4, []

        def load(r):
            at = r // Q * n + r % n
            y = xs[_span(t, T, r, 8), :].astype(f32) + ys[r % Q // n][at:at + 8]
            x_mid[r:r + 8, :] = y
            return y

        tasks = norm2_tasks(_Stream(), load)
        per = len(tasks) // 4
        for k in range(4):
            lhs = lambda i: jnp.concatenate(
                [h_o[_span(i, M // 2, (h * Q + k * n) // 2, n // 2), :] for h in range(2)], axis=0)
            ys.append(_strassen(lambda i: mx.dot(lhs(i), w_o[_span(i, 128), :]), _PAIRS_FIRST))
            mx.spread(tasks[k * per:(k + 1) * per], 600, 1100)
        mx.finish()

    def ffn(mx, v):
        def hidden(block):
            inner = lambda i, j: mx.dot(h_gu[_span(i, Q // 2), _span(j, 128)],
                                        w_gu[_span(block * 7 + i, 64), _span(j, 128)])
            return _strassen(lambda i: _strassen(partial(inner, i), (1, 3, 0, 2, 4, 5, 6)), _IN_ORDER)

        def tail_rows(z, u):
            low = lax.broadcasted_iota(i32, (16, 128), 1) < 64
            rows = [_tiles(z[r * Q + u * 16:r * Q + u * 16 + 16]) for r in range(4)]
            rolled = [[pltpu.roll(a, 64, 1) for a in row] for row in rows]
            yield
            act = [[jnp.maximum(jnp.where(low, a[p], ra[p + 1]), 0.0) * jnp.where(low, ra[p], a[p + 1])
                    for p in (0, 2)] for a, ra in zip(rows, rolled)]
            for r in range(2):
                h_dt[_span(r, Q // 2, u * 8, 8), :] = _pack(
                    jnp.concatenate(_lhs_ops(*act[r], *act[2 + r]), axis=1))
            yield [t for r in range(2) for t in _tiles(h_dt[_span(r, Q // 2, u * 8, 8), :])]

        tail = hidden(6)
        mx.spread([(1, (350,), partial(tail_rows, tail, u)) for u in range(Q // 16)], 300, 6000)
        for c in range(3):
            gate, up = hidden(2 * c), hidden(2 * c + 1)
            act = jnp.maximum(gate, 0.0) * up
            for i, inner in enumerate(_two_level(_lhs_ops, [act[r * Q:(r + 1) * Q] for r in range(4)])):
                for j, a in enumerate(_tiles(inner())):
                    h_dn[_span(i * 7 + j, Q // 2), _span(c, 128)] = _pack(a)

        def outer(i):
            rest = jnp.block([[mx.dot(h_dt[_span(r, Q // 2), _span(i, 128)], w_dt[_span(i, 64), _span(c, 128)])
                               for c in range(2)] for r in range(2)])
            inner = lambda j: mx.dot(h_dn[_span(i * 7 + j, Q // 2), :], w_dn[_span(i, 192), _span(j, 128)])
            return _strassen(inner, (1, 3, 2, 4, 0, 6, 5)) + rest

        y = _strassen(outer, _PAIRS_FIRST)
        mx.finish()
        for r, c in ((1, 0), (0, 1), (1, 1), (0, 0)):
            part = y[r * M:(r + 1) * M, c * 256:(c + 1) * 256] + x_mid[_span(r, M), _span(c, 256)]
            xs[_span(v % NT, T, r * M, M), _span(c, 256)] = part.astype(bf16)

    one = 7 * M
    for ref in (k_buf, v_buf):
        ref[0, :, :HALO, :] = jnp.zeros((4, HALO, 128), f32)
    get_qkv(0).wait()
    _run(qkv_weight_tasks(0), 600)

    get_x(0).wait()
    _run(norm1_tasks(_Stream(), 0), 1500)
    mx = stream()
    have = {i: qkv_product(mx, 0, 0, i) for i in (1, 3)}

    get_qkv(1).wait()
    mx = stream()
    mx.spread(qkv_weight_tasks(1), 100, 5 * M - 20)
    qkv(mx, 0, 0, have)
    mx.finish()

    get_qkv(2).wait()
    mx = stream()
    mx.spread(qkv_weight_tasks(2), 100, 4 * M - 20)
    have = {i: qkv_product(mx, 0, 1, i) for i in _IN_ORDER[:4]}
    mx.finish()

    get_x(1).wait()
    mx = stream()
    mx.spread(norm1_tasks(_Stream(), 1), 300, 1000)
    qkv(mx, 0, 1, have)
    mx.finish()

    get_x(2).wait()
    get_o.wait()
    mx = stream()
    mx.spread(_merge(norm1_tasks(_Stream(), 2), out_weight_tasks()), 300, one + 200)
    qkv(mx, 0, 2)
    tasks, hand_over = attention_tasks(mx, 0)
    mx.spread(tasks + hand_over, 200, 3 * one - 20)
    for j in range(3):
        qkv(mx, 1, j)
    mx.finish()

    get_g.wait()
    get_u.wait()
    gate_up, down = ffn_weight_tasks()
    mx = stream()
    mx.spread(gate_up[:28], 0, one)
    qkv(mx, 2, 0)
    mx.spread(gate_up[28:], 0, one - 20)
    load = project(mx, 0)
    mx.finish()
    for r in range(0, T, 8):
        load(r)

    get_x(3).wait()
    get_d.wait()
    mx = stream()
    mx.spread(norm2_tasks(_Stream(), lambda r: x_mid[r:r + 8, :]) + norm1_tasks(_Stream(), 3) + down,
              0, 2 * one - 20)
    qkv(mx, 2, 1)
    qkv(mx, 2, 2)
    mx.finish()

    @pl.loop(1, NV + 1)
    def _(v):
        mx = stream()
        tasks, hand_over = attention_tasks(mx, v)
        mx.spread(tasks, 400, 10976)
        mx.spread(hand_over, 10976, 16300)
        ffn(mx, v - 1)
        pl.when(v > NT)(lambda: put_x(v - 1 - NT).start())

        @pl.when(v < NV - 2)
        def _():
            mx = stream()
            tasks = norm1_tasks(mx, v + 3)
            mx.spread(tasks + norm2_tasks(mx, project(mx, v)), -1300, 5100)
            for j in range(3):
                qkv(mx, v + 2, j)
            mx.finish()

        @pl.when((v >= NV - 2) & (v < NV))
        def _():
            project_and_norm(stream(), v)

    for t in range(NT):
        put_x(t).wait()


@jax.jit
def pallas_interleave_layers__sliding_local_dilated__glu_gated_reglu__prompt_kernel(
    A_x: jax.Array,
    A_wqkv: jax.Array,
    A_wo: jax.Array,
    B_x: jax.Array,
    B_W_gate: jax.Array,
    B_W_up: jax.Array,
    B_W_down: jax.Array,
):
    del B_x
    assert A_x.shape == (1, S, D) and B_W_gate.shape == (D, F) and A_x.dtype == bf16
    vmem = pltpu.VMEM
    out = pl.pallas_call(
        _kernel,
        in_specs=[pl.BlockSpec(memory_space=pl.ANY)] * 6,
        out_specs=pl.BlockSpec(memory_space=pl.ANY),
        out_shape=jax.ShapeDtypeStruct((S, D), A_x.dtype),
        scratch_shapes=[
            vmem((S, D), bf16), vmem((T, D), f32),
            vmem((3, D, D), bf16), vmem((D, D), bf16),
            vmem((D, F), bf16), vmem((D, F), bf16), vmem((F, D), bf16), vmem((4, 560, 128), f32),
            vmem((21 * 128, 256), i32), vmem((7 * 128, 256), i32), vmem((49 * 64, 896), i32),
            vmem((7 * 192, 896), i32), vmem((7 * 64, 256), i32),
            vmem((NT * 7 * M // 2, 256), i32), vmem((7 * M // 2, 256), i32), vmem((7 * Q // 2, 896), i32),
            vmem((49 * Q // 2, 384), i32), vmem((M // 2, 896), i32),
            vmem((NT, 4, T, 128), f32), vmem((NT, 4, HALO + T, 128), f32), vmem((NT, 4, HALO + T, 128), f32),
            vmem((8, 128), i32), pltpu.SemaphoreType.DMA((9,)),
        ],
        compiler_params=pltpu.CompilerParams(vmem_limit_bytes=100 * 2**20),
    )(A_x.reshape(S, D), A_wqkv, A_wo, B_W_gate, B_W_up, B_W_down)
    return out.reshape(A_x.shape)
```

```python
import functools

import jax
import jax.numpy as jnp
from jax import lax
import jax.experimental.pallas as pl
import jax.experimental.pallas.tpu as pltpu

S, D, F = 2048, 512, 1792
DH, WIN, DIL = 16, 8, 2
EPS, MASKED = 1e-5, -1e9
LOG2E = 1.4426950408889634
T = 512
M, Q = T // 2, T // 4
NT = S // T
NV = 2 * NT
HALO = 16
SPREAD = 64.0
f32, bf16, i32 = jnp.float32, jnp.bfloat16, jnp.int32
partial = functools.partial


def _lhs_ops(a11, a12, a21, a22):
    return [a11 + a22, a21 + a22, a11, a22, a11 + a12, a21 - a11, a12 - a22]


def _rhs_ops(b11, b12, b21, b22):
    return [b11 + b22, b11, b12 - b22, b21 - b11, b22, b11 + b12, b21 + b22]


def _strassen(product, order):
    m = {i: product(i) for i in order}
    return jnp.block([[(m[3] - m[4]) + m[0] + m[6], m[2] + m[4]],
                      [m[1] + m[3], (m[2] - m[1]) + m[0] + m[5]]])


def _halves(*rows):
    return [h for r in rows for h in (r[:, :r.shape[1] // 2], r[:, r.shape[1] // 2:])]


def _two_level(ops, rows):
    top, bot = ops(*_halves(rows[0], rows[2])), ops(*_halves(rows[1], rows[3]))
    return [partial(lambda t, b: jnp.concatenate(ops(*_halves(t, b)), axis=1), t, b)
            for t, b in zip(top, bot)]


def _pack(x):
    return pltpu.bitcast(x.astype(bf16), i32)


def _tiles(x):
    return [x[:, c:c + 128] for c in range(0, x.shape[1], 128)]


def _span(i, n, start=0, size=None):
    at = i * n + start
    return pl.ds(at if isinstance(at, int) else pl.multiple_of(at, 8), n if size is None else size)


class _Stream:
    def __init__(self, never=None):
        self.never, self.clock, self.now, self.steps, self.results = never, 0.0, 0.0, [], []

    def spread(self, tasks, start, end):
        total, done = sum(w for w, _, _ in tasks), 0
        for weight, leads, make in tasks:
            done += weight
            due = self.clock + start + (end - start) * done / total
            slot = (end - start) * weight / total
            gen = make()
            self.steps += [(due - (lead * slot if lead < 1 else lead), gen) for lead in leads + (0,)]
        self.steps.sort(key=lambda step: step[0])

    def finish(self):
        for _, gen in self.steps:
            next(gen)
        self.steps = []

    def dot(self, a, b):
        n = a.shape[0] // 8
        cycles = a.shape[0] * (a.shape[1] // 128) * (b.shape[1] // 128) / 2
        ties = {}
        while self.steps and self.steps[0][0] < self.clock + cycles:
            self.now, gen = self.steps.pop(0)
            for v in next(gen) or []:
                ties.setdefault(max(0, int((self.now - self.clock) / cycles * n)), []).append(v)
        if ties:
            rows, at = [], 0
            for g in sorted(ties):
                bits = functools.reduce(
                    jnp.bitwise_or, [v if v.dtype == i32 else pltpu.bitcast(v, i32) for v in ties[g]])
                row = jnp.where(self.never, bits, a[g * 8:g * 8 + 8, :128])
                if a.shape[1] > 128:
                    row = jnp.concatenate([row, a[g * 8:g * 8 + 8, 128:]], axis=1)
                rows += ([a[at:g * 8]] if at < g * 8 else []) + [row]
                at = g * 8 + 8
            a = jnp.concatenate(rows + ([a[at:]] if at < n * 8 else []), axis=0)
        out = jnp.dot(pltpu.bitcast(a, bf16), pltpu.bitcast(b, bf16), preferred_element_type=f32)
        self.results += [(self.clock + 110 + 8 * r, out, r) for r in range(0, 2 * n, 4)]
        self.clock += cycles
        return out

    def not_before(self, x):
        ready = [r for r in self.results if r[0] <= self.now]
        if not ready:
            return x
        _, out, r = max(ready, key=lambda res: res[0])
        return jnp.where(self.never, out[r * 8:r * 8 + 8, :128], x)


def _step(weight, fn, *args):
    def gen():
        yield fn(*args)
    return weight, (), gen


def _merge(a, b):
    def keyed(tasks):
        total, done = sum(w for w, _, _ in tasks), 0
        for task in tasks:
            done += task[0]
            yield (done - task[0] / 2) / total, task
    return [task for _, task in sorted([*keyed(a), *keyed(b)], key=lambda kt: kt[0])]


def _run(tasks, cycles):
    plain = _Stream()
    plain.spread(tasks, 0, cycles)
    plain.finish()


_SEVEN_STEPS = tuple(k / 7 for k in range(6, 0, -1))
_IN_ORDER = (0, 1, 2, 5, 3, 4, 6)
_PAIRS_FIRST = (1, 3, 2, 4, 0, 5, 6)


def _put_one_level(ops, dst, block, n, u, top, bot):
    for i, v in enumerate(ops(*_halves(top, bot))):
        dst[_span(block + i, n, u * 8, 8), :] = _pack(v)
    return [t for i in range(7) for t in _tiles(dst[_span(block + i, n, u * 8, 8), :])]


def _put_two_level(ops, order, dst, block, n, at, rows):
    inner = _two_level(ops, rows)
    for i in order:
        dst[_span(block + i, n, at, 8), :] = _pack(inner[i]())
        yield _tiles(dst[_span(block + i, n, at, 8), 640:])


def _plain_layers(xs, wqkv, wo, wg, wu, wd, k_buf, v_buf):
    n = 64
    dot = lambda a, b: jnp.dot(a.astype(bf16), b, preferred_element_type=f32)

    def norm(x):
        x = x - jnp.mean(x, axis=-1, keepdims=True)
        return x * lax.rsqrt(jnp.mean(x * x, axis=-1, keepdims=True) + EPS)

    @pl.loop(0, 2 * S // n)
    def _(step):
        start = step % (S // n) * n
        rows = pl.ds(pl.multiple_of(start, n), n)
        x = xs[rows, :].astype(f32)
        h = norm(x)
        q, k, v = [jnp.stack(_tiles(dot(h, wqkv[j]))) for j in range(3)]
        for ref, new in ((k_buf, k), (v_buf, v)):
            ref[:, :HALO, :] = jnp.where(start == 0, new[:, :1], ref[:, n:n + HALO, :])
            ref[:, HALO:HALO + n, :] = new
        taps = lambda ref: jnp.stack([ref[:, pl.ds(HALO - DIL * w, n), :] for w in range(WIN)])
        prod = (q * taps(k_buf)).reshape(WIN * 4 * n, 128)
        same_head = (lax.broadcasted_iota(i32, (128, 128), 0) // DH
                     == lax.broadcasted_iota(i32, (128, 128), 1) // DH)
        head_sum = jnp.where(same_head, 1.0, 0.0).astype(bf16)
        s = dot(prod, head_sum) + dot(prod - prod.astype(bf16).astype(f32), head_sum)
        s = s.reshape(WIN, 4, n, 128) * DH ** -0.5
        pos = lax.broadcasted_iota(i32, s.shape, 2) + start
        s = jnp.where(pos >= DIL * lax.broadcasted_iota(i32, s.shape, 0), s, MASKED)
        p = jnp.exp(s - jnp.max(s, axis=0))
        o = jnp.sum(p * taps(v_buf), axis=0) / jnp.sum(p, axis=0)
        x = x + dot(jnp.concatenate([o[t] for t in range(4)], axis=1), wo[...])
        h = norm(x)

        def chunk(c, x):
            f = pl.ds(pl.multiple_of(c * 256, 256), 256)
            return x + dot(jnp.maximum(dot(h, wg[:, f]), 0.0) * dot(h, wu[:, f]), wd[f, :])
        xs[rows, :] = lax.fori_loop(0, F // 256, chunk, x).astype(bf16)


def _kernel(x_hbm, wqkv_hbm, wo_hbm, wg_hbm, wu_hbm, wd_hbm, out_hbm,
            xs, x_mid, raw_qkv, raw_o, raw_g, raw_u, raw_d, wo_rows,
            w_qkv, w_o, w_gu, w_dn, w_dt, h_qkv, h_o, h_gu, h_dn, h_dt,
            q_buf, k_buf, v_buf, zeros, var_range, sem):
    copy = pltpu.make_async_copy
    get_x = lambda t: copy(x_hbm.at[pl.ds(t * T, T)], xs.at[pl.ds(t * T, T)], sem.at[t])
    get_qkv = lambda j: copy(wqkv_hbm.at[:, pl.ds(j * D, D)], raw_qkv.at[j], sem.at[4 + j])
    get_o, get_d = copy(wo_hbm, raw_o, sem.at[2]), copy(wd_hbm, raw_d, sem.at[3])
    get_g, get_u = copy(wg_hbm, raw_g, sem.at[7]), copy(wu_hbm, raw_u, sem.at[7])
    put_x = lambda t: copy(xs.at[_span(t, T)], out_hbm.at[_span(t, T)], sem.at[8])
    for c in (get_qkv(0), get_x(0), get_qkv(1), get_qkv(2), get_x(1), get_x(2),
              get_o, get_g, get_u, get_d, get_x(3)):
        c.start()
    zeros[...] = jnp.zeros(zeros.shape, i32)
    stream = lambda: _Stream(zeros[...] != 0)
    var_range[:, 0] = jnp.full((5, 8, 128), jnp.inf, f32)
    var_range[:, 1] = jnp.zeros((5, 8, 128), f32)

    def qkv_weight_tasks(j):
        lane = lax.broadcasted_iota(i32, (D // 2, 128), 1)
        group, eighth, head = lane // 32, (lane // 8) % 4, lane % 8
        src = [jnp.take_along_axis(w, head * DH + ((eighth - a) % 4) * 4 + group, axis=1)
               for a, w in enumerate(_tiles(pltpu.bitcast(raw_qkv[j], i32)))]
        cols = []
        for i in range(4):
            col = src[3]
            for a in range(3):
                col = jnp.where(eighth == (a + i) % 4, src[a], col)
            cols.append(pltpu.roll(col, 128 - 8 * i, 1) if i else col)
        words = jnp.concatenate(cols, axis=1)
        band = lambda r: pltpu.bitcast(words[r:r + 8], bf16).astype(f32)
        vregs = lambda w: [w[r:r + 8] for r in range(0, D // 2, 8)]
        build = lambda u: _put_one_level(_rhs_ops, w_qkv, j * 7, 128, u, band(u * 8), band(128 + u * 8))
        return ([_step(200, vregs, w) for w in src] + [_step(100, vregs, w) for w in cols[1:]]
                + [_step(25, build, u) for u in range(16)])

    def out_weight_tasks():
        def stage(g):
            for h in range(g * 4, g * 4 + 4):
                wo_rows[:, h * 17:h * 17 + DH, :] = jnp.stack(
                    _tiles(raw_o[h * DH:(h + 1) * DH, :].astype(f32)))
            return [wo_rows[t, g * 68:g * 68 + 8, :] for t in range(4)]

        def band(i, group, e):
            dim = lambda a: 4 * i + (group if a + i < 4 else (group + 1) % 4)
            return jnp.block([[wo_rows[t, pl.ds(a * 8 * 17 + dim(a), 8, stride=17), :] for t in range(4)]
                              for a in (2 * e, 2 * e + 1)])

        def build(i, group, e):
            return _put_one_level(_rhs_ops, w_o, 0, 128, i * 8 + group * 2 + e,
                                  band(i, group, e), band(2 + i, group, e))[10:]

        return ([_step(50, stage, g) for g in range(8)]
                + [_step(40, build, i, group, e) for i in range(2) for group in range(4) for e in range(2)])

    def ffn_weight_tasks():
        put = partial(_put_two_level, _rhs_ops, (1, 5, 2, 4, 0, 3, 6))

        def gate_up(ref, block, c, u):
            return put(w_gu, block * 7, 64, u * 8,
                       [ref[_span(r, 128, u * 16, 16), _span(c, 512)].astype(f32) for r in range(4)])

        def gate_up_tail(u):
            low = lax.broadcasted_iota(i32, (8, 128), 1) < 64
            load = lambda ref, r: _tiles(pltpu.bitcast(ref[_span(r, 128, u * 16, 16), 1536:], i32))
            rows = [[(g, up, pltpu.roll(g, 64, 1), pltpu.roll(up, 64, 1))
                     for g, up in zip(load(raw_g, r), load(raw_u, r))] for r in range(4)]
            yield
            rows = [jnp.concatenate([z for g, up, rg, ru in row
                                     for z in (jnp.where(low, g, ru), jnp.where(low, rg, up))], axis=1)
                    for row in rows]
            yield from put(w_gu, 6 * 7, 64, u * 8, [pltpu.bitcast(row, bf16).astype(f32) for row in rows])

        def down(c, u):
            return put(w_dn, 0, 192, c * 64 + u * 8,
                       [raw_d[_span(c * 4 + r, 128, u * 16, 16), :].astype(f32) for r in range(4)])

        def down_tail(u):
            top, bot = [raw_d[_span(r, 128, u * 16, 16), :].astype(f32) for r in (12, 13)]
            return _put_one_level(_rhs_ops, w_dt, 0, 64, u, top, bot)[::2]

        return ([(200, _SEVEN_STEPS, partial(gate_up, ref, 2 * c + s, c, u))
                 for s, ref in enumerate((raw_g, raw_u)) for c in range(3) for u in range(8)]
                + [(200, (300,) + _SEVEN_STEPS, partial(gate_up_tail, u)) for u in range(8)],
                [(200, _SEVEN_STEPS, partial(down, c, u)) for c in range(3) for u in range(8)]
                + [_step(60, down_tail, u) for u in range(8)])

    def norm_tasks(mx, load, parts, last, stage):
        seen = []

        def rows(normed, r):
            x = load(r)
            lanes = _tiles(x)
            mean = jnp.sum(mx.not_before(lanes[0]) + lanes[1] + lanes[2] + lanes[3],
                           axis=-1, keepdims=True) * (1.0 / D)
            yield
            x = x - mean
            var = jnp.sum(x * x, axis=-1, keepdims=True) * (1.0 / D)
            yield
            normed[r] = x * lax.rsqrt(var + EPS)
            seen[:] = (jnp.minimum(seen[0], var), jnp.maximum(seen[1], var)) if seen else (var, var)
            yield [normed[r][:, :128]]

        def record():
            var_range[stage, 0] = jnp.minimum(var_range[stage, 0], seen[0])
            var_range[stage, 1] = jnp.maximum(var_range[stage, 1], seen[1])

        def bands(normed, starts):
            return [jnp.concatenate([normed[s], normed[s + 8]], axis=0) for s in starts]

        tasks = []
        for u in range(T // parts // 16):
            normed = {}
            starts = [p * (T // parts) + u * 16 for p in range(parts)]
            tasks += [(30, (450, 180), partial(rows, normed, r)) for s in starts for r in (s, s + 8)]
            tasks.append(last(u, partial(bands, normed, starts)))
        return tasks + [_step(0, record)]

    def norm1_tasks(mx, v):
        t = v % NT
        put = lambda u, bands: _put_one_level(_lhs_ops, h_qkv, t * 7, M // 2, u, *bands())
        load = lambda r: xs[_span(t, T, r, 8), :].astype(f32)
        return norm_tasks(mx, load, 2, partial(_step, 20, put), v // NT * 2)

    def norm2_tasks(mx, v, load):
        def put(u, bands):
            yield from _put_two_level(_lhs_ops, (2, 5, 1, 3, 0, 4, 6), h_gu, 0, Q // 2, u * 8, bands())
        return norm_tasks(mx, load, 4, lambda u, bands: (140, _SEVEN_STEPS, partial(put, u, bands)),
                          v // NT * 2 + 1)

    def qkv_product(mx, v, j, i):
        return mx.dot(h_qkv[_span(v % NT * 7 + i, M // 2), :], w_qkv[_span(j * 7 + i, 128), :])

    def qkv(mx, v, j, have=()):
        y = _strassen(lambda i: have[i] if i in have else qkv_product(mx, v, j, i), _IN_ORDER)
        if j == 0:
            q_buf[v % NT] = jnp.stack(_tiles(y * (DH ** -0.5 * LOG2E)))
        else:
            (k_buf, v_buf)[j - 1][v % NT, :, HALO:, :] = jnp.stack(_tiles(y))

    def attention_tasks(mx, v):
        t, t_next = v % NT, (v + 1) % NT

        def rows(result, r):
            tap = lambda ref, w: ref[t, :, pl.ds(HALO + r - DIL * w, 8), :]
            q = q_buf[t, :, r:r + 8, :]
            q = jnp.concatenate([mx.not_before(q[0])[None], q[1:]], axis=0)
            s = [jnp.sum(q * tap(k_buf, w), axis=0) for w in range(WIN)]
            rolled = [[pltpu.roll(z, shift, 1) for shift in (32, 64, 96)] for z in s]
            yield
            s = jnp.stack([(z + zr[0]) + (zr[1] + zr[2]) for z, zr in zip(s, rolled)])
            yield
            values = [tap(v_buf, w) for w in range(WIN)]
            if r < HALO:
                pos = lax.broadcasted_iota(i32, s.shape, 1) + (t * T + r)
                s = jnp.where(pos >= DIL * lax.broadcasted_iota(i32, s.shape, 0), s, MASKED * LOG2E)
                first = v_buf[t, :, HALO:HALO + 1, :]
                values = [jnp.where(pos[:4] >= DIL * w, z, first) if w else z for w, z in enumerate(values)]
            p = jnp.exp2(s - jnp.max(s, axis=0))
            o = functools.reduce(jnp.add, [p[w] * z for w, z in enumerate(values)])
            o = o * pl.reciprocal(jnp.sum(p, axis=0), full_range=False)
            result[r] = [o[i] for i in range(4)]
            yield result[r]

        def operands(result, u):
            top, bot = [jnp.block([result[r], result[r + 8]]) for r in (u * 16, M + u * 16)]
            return _put_one_level(_lhs_ops, h_o, 0, M // 2, u, top, bot)

        def hand_over():
            for ref in (k_buf, v_buf):
                ref[t_next, :, :HALO, :] = ref[t, :, T:, :]

        tasks = []
        for u in range(M // 16):
            result = {}
            tasks += [(162, (480, 60), partial(rows, result, s + u * 16 + e)) for s in (0, M) for e in (0, 8)]
            tasks.append(_step(34, operands, result, u))
        return tasks, [_step(1, hand_over)]

    def project(mx, v):
        y = _strassen(lambda i: mx.dot(h_o[_span(i, M // 2), :], w_o[_span(i, 128), :]), _IN_ORDER)
        y = xs[_span(v % NT, T), :].astype(f32) + y

        def load(r):
            x_mid[r:r + 8, :] = y[r:r + 8]
            return y[r:r + 8]
        return load

    def project_and_norm(mx, v):
        t, n, ys = v % NT, Q // 4, []

        def load(r):
            at = r // Q * n + r % n
            y = xs[_span(t, T, r, 8), :].astype(f32) + ys[r % Q // n][at:at + 8]
            x_mid[r:r + 8, :] = y
            return y

        tasks = norm2_tasks(_Stream(), v, load)
        per = len(tasks) // 4
        for k in range(4):
            lhs = lambda i: jnp.concatenate(
                [h_o[_span(i, M // 2, (h * Q + k * n) // 2, n // 2), :] for h in range(2)], axis=0)
            ys.append(_strassen(lambda i: mx.dot(lhs(i), w_o[_span(i, 128), :]), _PAIRS_FIRST))
            mx.spread(tasks[k * per:(k + 1) * per if k < 3 else None], 750, 1100)
        mx.finish()

    def ffn(mx, v):
        def hidden(block):
            inner = lambda i, j: mx.dot(h_gu[_span(i, Q // 2), _span(j, 128)],
                                        w_gu[_span(block * 7 + i, 64), _span(j, 128)])
            return _strassen(lambda i: _strassen(partial(inner, i), (1, 3, 0, 2, 4, 5, 6)), _IN_ORDER)

        def tail_rows(z, u):
            low = lax.broadcasted_iota(i32, (16, 128), 1) < 64
            rows = [_tiles(z[r * Q + u * 16:r * Q + u * 16 + 16]) for r in range(4)]
            rolled = [[pltpu.roll(a, 64, 1) for a in row] for row in rows]
            yield
            act = [[jnp.maximum(jnp.where(low, a[p], ra[p + 1]), 0.0) * jnp.where(low, ra[p], a[p + 1])
                    for p in (0, 2)] for a, ra in zip(rows, rolled)]
            for r in range(2):
                h_dt[_span(r, Q // 2, u * 8, 8), :] = _pack(
                    jnp.concatenate(_lhs_ops(*act[r], *act[2 + r]), axis=1))
            yield [t for r in range(2) for t in _tiles(h_dt[_span(r, Q // 2, u * 8, 8), :])]

        tail = hidden(6)
        mx.spread([(1, (350,), partial(tail_rows, tail, u)) for u in range(Q // 16)], 300, 6000)
        for c in range(3):
            gate, up = hidden(2 * c), hidden(2 * c + 1)
            act = jnp.maximum(gate, 0.0) * up
            for i, inner in enumerate(_two_level(_lhs_ops, [act[r * Q:(r + 1) * Q] for r in range(4)])):
                for j, a in enumerate(_tiles(inner())):
                    h_dn[_span(i * 7 + j, Q // 2), _span(c, 128)] = _pack(a)

        def outer(i):
            rest = jnp.block([[mx.dot(h_dt[_span(r, Q // 2), _span(i, 128)], w_dt[_span(i, 64), _span(c, 128)])
                               for c in range(2)] for r in range(2)])
            inner = lambda j: mx.dot(h_dn[_span(i * 7 + j, Q // 2), :], w_dn[_span(i, 192), _span(j, 128)])
            return _strassen(inner, (1, 3, 2, 4, 0, 6, 5)) + rest

        y = _strassen(outer, _PAIRS_FIRST)
        mx.finish()
        for r, c in ((1, 0), (0, 1), (1, 1), (0, 0)):
            part = y[r * M:(r + 1) * M, c * 256:(c + 1) * 256] + x_mid[_span(r, M), _span(c, 256)]
            xs[_span(v % NT, T, r * M, M), _span(c, 256)] = part.astype(bf16)

    one = 7 * M
    for ref in (k_buf, v_buf):
        ref[0, :, :HALO, :] = jnp.zeros((4, HALO, 128), f32)
    get_qkv(0).wait()
    _run(qkv_weight_tasks(0), 600)

    get_x(0).wait()
    _run(norm1_tasks(_Stream(), 0), 1500)
    mx = stream()
    have = {i: qkv_product(mx, 0, 0, i) for i in (1, 3)}

    get_qkv(1).wait()
    mx = stream()
    mx.spread(qkv_weight_tasks(1), 100, 5 * M - 20)
    qkv(mx, 0, 0, have)
    mx.finish()

    get_qkv(2).wait()
    mx = stream()
    mx.spread(qkv_weight_tasks(2), 100, 4 * M - 20)
    have = {i: qkv_product(mx, 0, 1, i) for i in _IN_ORDER[:4]}
    mx.finish()

    get_x(1).wait()
    mx = stream()
    mx.spread(norm1_tasks(_Stream(), 1), 300, 1000)
    qkv(mx, 0, 1, have)
    mx.finish()

    get_x(2).wait()
    get_o.wait()
    mx = stream()
    mx.spread(_merge(norm1_tasks(_Stream(), 2), out_weight_tasks()), 300, one + 200)
    qkv(mx, 0, 2)
    tasks, hand_over = attention_tasks(mx, 0)
    mx.spread(tasks + hand_over, 200, 3 * one - 20)
    for j in range(3):
        qkv(mx, 1, j)
    mx.finish()

    get_g.wait()
    get_u.wait()
    gate_up, down = ffn_weight_tasks()
    mx = stream()
    mx.spread(gate_up[:28], 0, one)
    qkv(mx, 2, 0)
    mx.spread(gate_up[28:], 0, one - 20)
    load = project(mx, 0)
    mx.finish()
    for r in range(0, T, 8):
        load(r)

    get_x(3).wait()
    get_d.wait()
    mx = stream()
    mx.spread(norm2_tasks(_Stream(), 0, lambda r: x_mid[r:r + 8, :]) + norm1_tasks(_Stream(), 3) + down,
              0, 2 * one - 20)
    qkv(mx, 2, 1)
    qkv(mx, 2, 2)
    mx.finish()

    @pl.loop(1, NV + 1)
    def _(v):
        mx = stream()
        tasks, hand_over = attention_tasks(mx, v)
        mx.spread(tasks, 400, 10976)
        mx.spread(hand_over, 10976, 16300)
        ffn(mx, v - 1)
        pl.when(v > NT)(lambda: put_x(v - 1 - NT).start())

        @pl.when(v < NV - 2)
        def _():
            mx = stream()
            tasks = norm1_tasks(mx, v + 3)
            mx.spread(tasks + norm2_tasks(mx, v, project(mx, v)), -1300, 5100)
            for j in range(3):
                qkv(mx, v + 2, j)
            mx.finish()

        @pl.when((v >= NV - 2) & (v < NV))
        def _():
            project_and_norm(stream(), v)

    lo = [jnp.min(var_range[i, 0], axis=0, keepdims=True) for i in range(4)]
    hi = [jnp.max(var_range[i, 1], axis=0, keepdims=True) for i in range(4)]
    even = SPREAD * lo[0] * (hi[0] + EPS) >= hi[0] * (lo[0] + EPS)
    for i in range(1, 4):
        even &= SPREAD * (lo[i] + EPS) >= jnp.maximum(hi[i], hi[i - 1])
    uneven = jnp.max(jnp.where(even, 0.0, 1.0)) > 0.0
    for t in range(NT):
        put_x(t).wait()

    @pl.when(uneven)
    def _():
        whole = copy(x_hbm, xs, sem.at[0])
        whole.start()
        whole.wait()
        _plain_layers(xs, raw_qkv, raw_o, raw_g, raw_u, raw_d, k_buf.at[0], v_buf.at[0])
        whole = copy(xs, out_hbm, sem.at[0])
        whole.start()
        whole.wait()


@jax.jit
def pallas_interleave_layers__sliding_local_dilated__glu_gated_reglu__prompt_kernel(
    A_x: jax.Array,
    A_wqkv: jax.Array,
    A_wo: jax.Array,
    B_x: jax.Array,
    B_W_gate: jax.Array,
    B_W_up: jax.Array,
    B_W_down: jax.Array,
):
    del B_x
    assert A_x.shape == (1, S, D) and B_W_gate.shape == (D, F) and A_x.dtype == bf16
    vmem = pltpu.VMEM
    out = pl.pallas_call(
        _kernel,
        in_specs=[pl.BlockSpec(memory_space=pl.ANY)] * 6,
        out_specs=pl.BlockSpec(memory_space=pl.ANY),
        out_shape=jax.ShapeDtypeStruct((S, D), A_x.dtype),
        scratch_shapes=[
            vmem((S, D), bf16), vmem((T, D), f32),
            vmem((3, D, D), bf16), vmem((D, D), bf16),
            vmem((D, F), bf16), vmem((D, F), bf16), vmem((F, D), bf16), vmem((4, 560, 128), f32),
            vmem((21 * 128, 256), i32), vmem((7 * 128, 256), i32), vmem((49 * 64, 896), i32),
            vmem((7 * 192, 896), i32), vmem((7 * 64, 256), i32),
            vmem((NT * 7 * M // 2, 256), i32), vmem((7 * M // 2, 256), i32), vmem((7 * Q // 2, 896), i32),
            vmem((49 * Q // 2, 384), i32), vmem((M // 2, 896), i32),
            vmem((NT, 4, T, 128), f32), vmem((NT, 4, HALO + T, 128), f32), vmem((NT, 4, HALO + T, 128), f32),
            vmem((8, 128), i32), vmem((5, 2, 8, 128), f32), pltpu.SemaphoreType.DMA((9,)),
        ],
        compiler_params=pltpu.CompilerParams(vmem_limit_bytes=100 * 2**20),
    )(A_x.reshape(S, D), A_wqkv, A_wo, B_W_gate, B_W_up, B_W_down)
    return out.reshape(A_x.shape)
```
